```python
import jax
import jax.numpy as jnp

def _softmax(x, axis=-1):
    return jax.nn.softmax(x, axis=axis)
def _gelu(x):
    return jax.nn.gelu(x, approximate=True)
def _silu(x):
    return jax.nn.silu(x)
def _sigmoid(x):
    return jax.nn.sigmoid(x)
def _layernorm(x, axis=-1, eps=1e-5):
    m = jnp.mean(x, axis=axis, keepdims=True)
    v = jnp.var(x, axis=axis, keepdims=True)
    return (x - m) / jnp.sqrt(v + eps)
def _scatter_add(tgt, idx, src, axis=0):
    return tgt.at[idx].add(src)
def _segment_sum(src, seg, n):
    return jax.ops.segment_sum(src, seg, n)
class _Rng:
    def __init__(self, key):
        self._k = key
    def _next(self):
        self._k, sub = jax.random.split(self._k)
        return sub
    def normal(self, shape):
        return jax.random.normal(self._next(), shape, dtype=jnp.bfloat16)
    def randint(self, lo, hi, shape):
        return jax.random.randint(self._next(), shape, lo, hi, dtype=jnp.int32)
    def uniform(self, shape, lo=0.0, hi=1.0):
        return jax.random.uniform(self._next(), shape, jnp.bfloat16, lo, hi)
    def permutation(self, n):
        return jax.random.permutation(self._next(), n)


kernel_name = 'sequential_preLN__sliding_block_cached__glu_gated_swiglu__decode'

def setup_inputs():
    _rng = _Rng(jax.random.key(int.from_bytes(__import__("os").urandom(4), "little")))
    _w = (lambda a: (lambda t: t.astype(jnp.bfloat16) if jnp.issubdtype(t.dtype, jnp.floating) else t)(jnp.asarray(a)))
    def _A_setup():
        B, Sq, D = 1, 1, 640
        Hq, Hkv, Sk, Dh = 32, 32, 32768, 192
        assert Hq % Hkv == 0, (Hq, Hkv)
        return {
            "x": _w((lambda *s: _rng.normal(s) * 0.05)(B, Sq, D)),
            "k_cache": _w((lambda *s: _rng.normal(s) * 0.05)(B, Hkv, Sk, Dh)),
            "v_cache": _w((lambda *s: _rng.normal(s) * 0.05)(B, Hkv, Sk, Dh)),
            "wq": _w((lambda *s: _rng.normal(s) * 0.05)(D, Hq * Dh) * (D ** -0.5)),
            "wo": _w((lambda *s: _rng.normal(s) * 0.05)(Hq * Dh, D) * ((Hq * Dh) ** -0.5)),
        }
    _A_in = _A_setup()

    def _B_setup():
        B, S, D, F = 1, 1, 640, 1536
        return {
            "x": _w((lambda *s: _rng.normal(s) * 0.05)(B, S, D)),
            "w1": _w((lambda *s: _rng.normal(s) * 0.05)(D, F) * (2.0 / D) ** 0.5),
            "w3": _w((lambda *s: _rng.normal(s) * 0.05)(D, F) * (2.0 / D) ** 0.5),
            "w2": _w((lambda *s: _rng.normal(s) * 0.05)(F, D) * (2.0 / F) ** 0.5),
        }
    _B_in = _B_setup()

    return {
        "A_x": _A_in["x"],
        "A_k_cache": _A_in["k_cache"],
        "A_v_cache": _A_in["v_cache"],
        "A_wq": _A_in["wq"],
        "A_wo": _A_in["wo"],
        "B_x": _B_in["x"],
        "B_w1": _B_in["w1"],
        "B_w3": _B_in["w3"],
        "B_w2": _B_in["w2"],
    }

def reference(A_x, A_k_cache, A_v_cache, A_wq, A_wo, B_x, B_w1, B_w3, B_w2):
    def _A_ref(x, k_cache, v_cache, wq, wo):
        B, Sq, D = x.shape
        Hq, Dh = 32, 192
        Hkv, Sk = k_cache.shape[1], k_cache.shape[2]
        W = min(4096, max(256, Sk // 4))
        rep = Hq // Hkv
        q = (lambda x, *d: x.transpose(*d))((x @ wq).reshape(B, Sq, Hq, Dh), 0, 2, 1, 3)
        k = jnp.repeat(k_cache[:, :, Sk - W:, :], rep, axis=1)
        v = jnp.repeat(v_cache[:, :, Sk - W:, :], rep, axis=1)
        scores = jnp.einsum("bhqd,bhkd->bhqk", q, k) * (Dh ** -0.5)
        p = _softmax(scores, axis=-1)
        o = jnp.einsum("bhqk,bhkd->bhqd", p, v)
        return (lambda x, *d: x.transpose(*d))(o, 0, 2, 1, 3).reshape(B, Sq, Hq * Dh) @ wo

    def _B_ref(x, w1, w3, w2):
        gate = jnp.einsum("bsd,df->bsf", x, w1)
        up = jnp.einsum("bsd,df->bsf", x, w3)
        h = _silu(gate) * up
        out = jnp.einsum("bsf,fd->bsd", h, w2)
        return out

    x = A_x
    h = x + _A_ref(_layernorm(x, axis=-1), A_k_cache, A_v_cache, A_wq, A_wo)
    h2 = h + _B_ref(_layernorm(h, axis=-1), B_w1, B_w3, B_w2)
    return h2
```

```python
import functools
import jax
import jax.numpy as jnp
from jax import lax
import jax.experimental.pallas as pl
import jax.experimental.pallas.tpu as pltpu

H, DH, SK, D, F = 32, 192, 32768, 640, 1536
W = min(4096, max(256, SK // 4))
BF = jnp.bfloat16
F32 = jnp.float32


def _ln(x32):
    m = jnp.mean(x32, axis=-1, keepdims=True)
    c = x32 - m
    v = jnp.mean(c * c, axis=-1, keepdims=True)
    mb = m.astype(BF).astype(F32)
    vb = v.astype(BF).astype(F32)
    num = (x32 - mb).astype(BF).astype(F32)
    den = (vb + 1e-5).astype(BF).astype(F32)
    den = jnp.sqrt(den).astype(BF).astype(F32)
    return (num / den).astype(BF)


def make_kernel(NK=3, NV=3, NWO=3, wq_chunks=5, w_chunks=5, w2_chunks=4, compute=True, prio=False):
    DC = D // wq_chunks
    DC2 = D // w_chunks
    FC = F // w2_chunks

    def kernel(x_hbm, kt_hbm, vt_hbm, wq_hbm, wo_hbm, w1_hbm, w3_hbm, w2_hbm, o_ref,
               x_v, wq_v, q_v, kbuf, vbuf, wobuf, w1_v, w3_v, w2_v,
               sem_x, sem_wq, sem_k, sem_v, sem_wo, sem_w1, sem_w3, sem_w2):
        def cp_x():
            return pltpu.make_async_copy(x_hbm, x_v, sem_x)
        def cp_wq(c):
            return pltpu.make_async_copy(wq_hbm.at[pl.ds(c * DC, DC)], wq_v.at[pl.ds(c * DC, DC)], sem_wq.at[c])
        def cp_k(h, slot):
            return pltpu.make_async_copy(kt_hbm.at[h, :, pl.ds(SK - W, W)], kbuf.at[slot], sem_k.at[slot])
        def cp_v(h, slot):
            return pltpu.make_async_copy(vt_hbm.at[h, :, pl.ds(SK - W, W)], vbuf.at[slot], sem_v.at[slot])
        def cp_wo(h, slot):
            return pltpu.make_async_copy(wo_hbm.at[pl.ds(pl.multiple_of(h * DH, DH), DH)], wobuf.at[slot], sem_wo.at[slot])
        def cp_w1(c):
            return pltpu.make_async_copy(w1_hbm.at[pl.ds(c * DC2, DC2)], w1_v.at[pl.ds(c * DC2, DC2)], sem_w1.at[c])
        def cp_w3(c):
            return pltpu.make_async_copy(w3_hbm.at[pl.ds(c * DC2, DC2)], w3_v.at[pl.ds(c * DC2, DC2)], sem_w3.at[c])
        def cp_w2(c):
            return pltpu.make_async_copy(w2_hbm.at[pl.ds(c * FC, FC)], w2_v.at[pl.ds(c * FC, FC)], sem_w2.at[c])

        cp_x().start()
        for c in range(wq_chunks):
            cp_wq(c).start()
        NPRE = min(NK, NV, NWO)
        for h in range(NPRE):
            cp_k(h, h).start()
            cp_v(h, h).start()
            cp_wo(h, h).start()

        cp_x().wait()
        x32 = x_v[...].astype(F32)
        lnx = _ln(x32)
        lnx8 = jnp.broadcast_to(lnx, (8, D))
        q = None
        for c in range(wq_chunks):
            cp_wq(c).wait()
            part = jnp.dot(lnx8[:, c * DC:(c + 1) * DC], wq_v[c * DC:(c + 1) * DC, :], preferred_element_type=F32)
            q = part if q is None else q + part
        for h in range(H):
            q_v[h] = q[:, h * DH:(h + 1) * DH]

        scale = jnp.float32(DH ** -0.5).astype(BF).astype(F32)

        def head(h, attn):
            slot = h % NK
            cp_k(h, slot).wait()
            if compute:
                qh = q_v[h].astype(BF)
                s = jnp.dot(qh, kbuf[slot], preferred_element_type=F32)
            @pl.when(h + NPRE < H)
            def _():
                cp_k(h + NPRE, slot).start()
            @pl.when(h + NPRE == H)
            def _():
                for c in range(w_chunks):
                    cp_w1(c).start()
            @pl.when(h + NPRE == H + 1)
            def _():
                for c in range(w_chunks):
                    cp_w3(c).start()
            @pl.when(h + NPRE == H + 2)
            def _():
                for c in range(w2_chunks):
                    cp_w2(c).start()
            if compute:
                s = s.astype(BF).astype(F32)
                s = (s * scale).astype(BF).astype(F32)
                m = jnp.max(s, axis=-1, keepdims=True)
                e = jnp.exp((s - m).astype(BF).astype(F32)).astype(BF).astype(F32)
                l = jnp.sum(e, axis=-1, keepdims=True).astype(BF).astype(F32)
                p = (e / l).astype(BF)
            cp_v(h, slot).wait()
            if compute:
                o = lax.dot_general(p, vbuf[slot], (((1,), (1,)), ((), ())), preferred_element_type=F32)
            @pl.when(h + NPRE < H)
            def _():
                cp_v(h + NPRE, slot).start()
            cp_wo(h, slot).wait()
            if compute:
                attn = attn + jnp.dot(o.astype(BF), wobuf[slot], preferred_element_type=F32)
            @pl.when(h + NPRE < H)
            def _():
                cp_wo(h + NPRE, slot).start()
            return attn

        attn = lax.fori_loop(0, H, head, jnp.zeros((8, D), F32))
        hres = (x32 + attn.astype(BF).astype(F32)).astype(BF).astype(F32)
        lnh = _ln(hres)
        gate = None
        up = None
        for c in range(w_chunks):
            cp_w1(c).wait()
            part = jnp.dot(lnh[:, c * DC2:(c + 1) * DC2], w1_v[c * DC2:(c + 1) * DC2, :], preferred_element_type=F32)
            gate = part if gate is None else gate + part
        for c in range(w_chunks):
            cp_w3(c).wait()
            part = jnp.dot(lnh[:, c * DC2:(c + 1) * DC2], w3_v[c * DC2:(c + 1) * DC2, :], preferred_element_type=F32)
            up = part if up is None else up + part
        gate = gate.astype(BF).astype(F32)
        up = up.astype(BF).astype(F32)
        sg = jax.nn.sigmoid(gate).astype(BF).astype(F32)
        hm = ((gate * sg).astype(BF).astype(F32) * up).astype(BF)
        out = None
        for c in range(w2_chunks):
            cp_w2(c).wait()
            part = jnp.dot(hm[:, c * FC:(c + 1) * FC], w2_v[c * FC:(c + 1) * FC, :], preferred_element_type=F32)
            out = part if out is None else out + part
        res = hres + out.astype(BF).astype(F32)
        o_ref[...] = res[0:1, :].astype(o_ref.dtype)

    @jax.jit
    def run(A_x, A_k_cache, A_v_cache, A_wq, A_wo, B_x, B_w1, B_w3, B_w2):
        x = A_x.reshape(1, D)
        kt = jnp.swapaxes(A_k_cache.reshape(H, SK, DH), 1, 2)
        vt = jnp.swapaxes(A_v_cache.reshape(H, SK, DH), 1, 2)
        out = pl.pallas_call(
            kernel,
            out_shape=jax.ShapeDtypeStruct((1, D), BF),
            in_specs=[pl.BlockSpec(memory_space=pl.ANY)] * 8,
            out_specs=pl.BlockSpec(memory_space=pltpu.VMEM),
            scratch_shapes=[
                pltpu.VMEM((1, D), BF),
                pltpu.VMEM((D, H * DH), BF),
                pltpu.VMEM((H, 8, DH), F32),
                pltpu.VMEM((NK, DH, W), BF),
                pltpu.VMEM((NV, DH, W), BF),
                pltpu.VMEM((NWO, DH, D), BF),
                pltpu.VMEM((D, F), BF),
                pltpu.VMEM((D, F), BF),
                pltpu.VMEM((F, D), BF),
                pltpu.SemaphoreType.DMA(()),
                pltpu.SemaphoreType.DMA((wq_chunks,)),
                pltpu.SemaphoreType.DMA((NK,)),
                pltpu.SemaphoreType.DMA((NV,)),
                pltpu.SemaphoreType.DMA((NWO,)),
                pltpu.SemaphoreType.DMA((w_chunks,)),
                pltpu.SemaphoreType.DMA((w_chunks,)),
                pltpu.SemaphoreType.DMA((w2_chunks,)),
            ],
            compiler_params=pltpu.CompilerParams(vmem_limit_bytes=100 * 1024 * 1024),
        )(x, kt, vt, A_wq, A_wo, B_w1, B_w3, B_w2)
        return out.reshape(1, 1, D)
    return run


pallas_sequential_preLN__sliding_block_cached__glu_gated_swiglu__decode_kernel = make_kernel(NK=3, NV=3, NWO=3)
```

```python
import functools
import jax
import jax.numpy as jnp
from jax import lax
import jax.experimental.pallas as pl
import jax.experimental.pallas.tpu as pltpu

H, DH, SK, D, F = 32, 192, 32768, 640, 1536
W = min(4096, max(256, SK // 4))
BF = jnp.bfloat16
F32 = jnp.float32


def _ln(x32):
    m = jnp.mean(x32, axis=-1, keepdims=True)
    c = x32 - m
    v = jnp.mean(c * c, axis=-1, keepdims=True)
    mb = m.astype(BF).astype(F32)
    vb = v.astype(BF).astype(F32)
    num = (x32 - mb).astype(BF).astype(F32)
    den = (vb + 1e-5).astype(BF).astype(F32)
    den = jnp.sqrt(den).astype(BF).astype(F32)
    return (num / den).astype(BF)


def pieces(R, C, pr, pc, order="cr", r0=0):
    rs = [(r0 + r, min(pr, R - r)) for r in range(0, R, pr)]
    cs = [(c, min(pc, C - c)) for c in range(0, C, pc)]
    if order == "rc":
        return [(r, nr, c, nc) for (r, nr) in rs for (c, nc) in cs]
    return [(r, nr, c, nc) for (c, nc) in cs for (r, nr) in rs]


def interleave(a, b):
    out = []
    for i in range(max(len(a), len(b))):
        if i < len(a): out.append(a[i])
        if i < len(b): out.append(b[i])
    return out


def split_even(lst, fracs):
    tot = sum(fracs)
    out, acc, prev = [], 0, 0
    for f in fracs:
        acc += f
        nxt = round(len(lst) * acc / tot)
        out.append(lst[prev:nxt]); prev = nxt
    return out


def make_kernel(R=3, kv_piece=(48, 512, "cr"), wq_piece=(8, 3072, "rc"), wo_piece=(32, 640, "rc"),
                w1_piece=(8, 1536, "rc"), w2_piece=(32, 640, "rc"), nq=4, n13=5, n2=4, wsplit=None,
                dual=True, nosem=False, wq_halves=True, nocomp=False):
    kvp = pieces(DH, W, *kv_piece)
    wop = pieces(DH, D, *wo_piece)
    P1 = 1 if dual else 0
    if wq_halves:
        top = pieces(D // 2, H * DH, *wq_piece)
        bot = pieces(D // 2, H * DH, *wq_piece, r0=D // 2)
        wqp = interleave([(p, 0) for p in top], [(p, 1) for p in bot])
    else:
        wqp = [(p, i % 2) for i, p in enumerate(pieces(D, H * DH, *wq_piece))]
    DC = D // n13
    FC = F // n2
    if wsplit is None:
        wsplit = [1] * (R - 1) + [3]

    def dot(a, b_ref_val_fn, shape, dims=(((1,), (0,)), ((), ()))):
        if nocomp:
            return jnp.zeros(shape, F32)
        return lax.dot_general(a, b_ref_val_fn(), dims, preferred_element_type=F32)

    def kernel(x_hbm, kt_hbm, vt_hbm, wq_hbm, wo_hbm, w1_hbm, w3_hbm, w2_hbm, o_ref,
               x_v, wq_v, q_v, kbuf, vbuf, wobuf, w1_v, w3_v, w2_v,
               sem_x, sem_wq, sem_k, sem_v, sem_wo, sem_w1, sem_w3, sem_w2):
        def cp2(src, dst, sem, p):
            r, nr, c, nc = p
            return pltpu.make_async_copy(src.at[pl.ds(r, nr), pl.ds(c, nc)], dst.at[pl.ds(r, nr), pl.ds(c, nc)], sem)
        def head_jobs(h, slot):
            ksrc = kt_hbm.at[h, :, pl.ds(SK - W, W)]
            vsrc = vt_hbm.at[h, :, pl.ds(SK - W, W)]
            wsrc = wo_hbm.at[pl.ds(pl.multiple_of(h * DH, DH), DH)]
            jobs = []
            for p in kvp:
                jobs.append((ksrc, kbuf.at[slot], sem_k.at[slot], p, 0))
                jobs.append((vsrc, vbuf.at[slot], sem_v.at[slot], p, P1))
            for i, p in enumerate(wop):
                jobs.append((wsrc, wobuf.at[slot], sem_wo.at[slot], p, P1 * (i % 2)))
            return jobs
        def run_jobs(jobs):
            for (a, b, s_, p, pr) in jobs:
                cp2(a, b, s_, p).start(priority=pr)
        def wait_all(ref, sem):
            pltpu.make_async_copy(ref, ref, sem).wait()

        pltpu.make_async_copy(x_hbm, x_v, sem_x).start()
        run_jobs([(wq_hbm, wq_v, sem_wq, p, P1 * t) for (p, t) in wqp])
        run_jobs(head_jobs(0, 0))
        wait_all(x_v, sem_x)
        x32 = x_v[...].astype(F32)
        lnx = _ln(x32)
        lnx8 = jnp.broadcast_to(lnx, (8, D))
        wait_all(wq_v, sem_wq)
        rest = []
        for h in range(1, R):
            rest += head_jobs(h, h)
        groups = split_even(rest, [1] * nq)
        QC = H // nq
        fences = [(kbuf.at[0], sem_k.at[0]), (vbuf.at[0], sem_v.at[0]), (wobuf.at[0], sem_wo.at[0])]
        fenced = set()
        for c in range(nq):
            qc = dot(lnx8, lambda: wq_v[:, c * QC * DH:(c + 1) * QC * DH], (8, QC * DH))
            for j in range(QC):
                q_v[c * QC + j] = qc[:, j * DH:(j + 1) * DH]
            run_jobs(groups[c])
            if c < len(fences) and c < nq - 1:
                wait_all(*fences[c]); fenced.add(c)

        scale = jnp.float32(DH ** -0.5).astype(BF).astype(F32)

        def head_compute(h, slot, attn, skip=()):
            if 0 not in skip: wait_all(kbuf.at[slot], sem_k.at[slot])
            if 1 not in skip: wait_all(vbuf.at[slot], sem_v.at[slot])
            if 2 not in skip: wait_all(wobuf.at[slot], sem_wo.at[slot])
            qh = q_v[h].astype(BF)
            s = dot(qh, lambda: kbuf[slot], (8, W))
            s = s.astype(BF).astype(F32)
            s = (s * scale).astype(BF).astype(F32)
            m = jnp.max(s, axis=-1, keepdims=True)
            e = jnp.exp((s - m).astype(BF).astype(F32)).astype(BF).astype(F32)
            l = jnp.sum(e, axis=-1, keepdims=True).astype(BF).astype(F32)
            p = (e / l).astype(BF)
            o = dot(p, lambda: vbuf[slot], (8, DH), (((1,), (1,)), ((), ())))
            return attn + dot(o.astype(BF), lambda: wobuf[slot], (8, D))

        attn = head_compute(0, 0, jnp.zeros((8, D), F32), skip=fenced)
        run_jobs(head_jobs(R, 0))

        def head(h, attn):
            slot = h % R
            attn = head_compute(h, slot, attn)
            run_jobs(head_jobs(h + R, slot))
            return attn

        attn = lax.fori_loop(1, H - R, head, attn)
        wjobs = []
        for c in range(n13):
            pp = pieces(DC, F, *w1_piece, r0=c * DC)
            wjobs += interleave([(w1_hbm, w1_v, sem_w1.at[c], p, 0) for p in pp],
                                [(w3_hbm, w3_v, sem_w3.at[c], p, P1) for p in pp])
        for c in range(n2):
            pp = pieces(FC, D, *w2_piece, r0=c * FC)
            wjobs += [(w2_hbm, w2_v, sem_w2.at[c], p, P1 * (i % 2)) for i, p in enumerate(pp)]
        wg = split_even(wjobs, wsplit)
        for i in range(R):
            h = H - R + i
            attn = head_compute(h, h % R, attn)
            if i == R - 1:
                hres = (x32 + attn.astype(BF).astype(F32)).astype(BF).astype(F32)
                lnh = _ln(hres)
            run_jobs(wg[i])
        gate = up = None
        for c in range(n13):
            rows = pl.ds(c * DC, DC)
            wait_all(w1_v.at[rows], sem_w1.at[c])
            wait_all(w3_v.at[rows], sem_w3.at[c])
            lc = lnh[:, c * DC:(c + 1) * DC]
            g_ = dot(lc, lambda: w1_v[c * DC:(c + 1) * DC, :], (8, F))
            u_ = dot(lc, lambda: w3_v[c * DC:(c + 1) * DC, :], (8, F))
            gate = g_ if gate is None else gate + g_
            up = u_ if up is None else up + u_
        gate = gate.astype(BF).astype(F32)
        up = up.astype(BF).astype(F32)
        sg = jax.nn.sigmoid(gate).astype(BF).astype(F32)
        hm = ((gate * sg).astype(BF).astype(F32) * up).astype(BF)
        out = None
        for c in range(n2):
            wait_all(w2_v.at[pl.ds(c * FC, FC)], sem_w2.at[c])
            o_ = dot(hm[:, c * FC:(c + 1) * FC], lambda: w2_v[c * FC:(c + 1) * FC, :], (8, D))
            out = o_ if out is None else out + o_
        res = hres + out.astype(BF).astype(F32)
        o_ref[...] = res[0:1, :].astype(o_ref.dtype)

    @jax.jit
    def run(A_x, A_k_cache, A_v_cache, A_wq, A_wo, B_x, B_w1, B_w3, B_w2):
        x = A_x.reshape(1, D)
        kt = jnp.swapaxes(A_k_cache.reshape(H, SK, DH), 1, 2)
        vt = jnp.swapaxes(A_v_cache.reshape(H, SK, DH), 1, 2)
        out = pl.pallas_call(
            kernel,
            out_shape=jax.ShapeDtypeStruct((1, D), BF),
            in_specs=[pl.BlockSpec(memory_space=pl.ANY)] * 8,
            out_specs=pl.BlockSpec(memory_space=pltpu.VMEM),
            scratch_shapes=[
                pltpu.VMEM((1, D), BF),
                pltpu.VMEM((D, H * DH), BF),
                pltpu.VMEM((H, 8, DH), F32),
                pltpu.VMEM((R, DH, W), BF),
                pltpu.VMEM((R, DH, W), BF),
                pltpu.VMEM((R, DH, D), BF),
                pltpu.VMEM((D, F), BF),
                pltpu.VMEM((D, F), BF),
                pltpu.VMEM((F, D), BF),
                pltpu.SemaphoreType.DMA(()),
                pltpu.SemaphoreType.DMA(()),
                pltpu.SemaphoreType.DMA((R,)),
                pltpu.SemaphoreType.DMA((R,)),
                pltpu.SemaphoreType.DMA((R,)),
                pltpu.SemaphoreType.DMA((n13,)),
                pltpu.SemaphoreType.DMA((n13,)),
                pltpu.SemaphoreType.DMA((n2,)),
            ],
            compiler_params=pltpu.CompilerParams(vmem_limit_bytes=100 * 1024 * 1024,
                                                 disable_semaphore_checks=nosem, disable_bounds_checks=nosem),
        )(x, kt, vt, A_wq, A_wo, B_w1, B_w3, B_w2)
        return out.reshape(1, 1, D)
    return run


pallas_sequential_preLN__sliding_block_cached__glu_gated_swiglu__decode_kernel = make_kernel(kv_piece=(24, 512, "cr"))
```

```python
import functools
import jax
import jax.numpy as jnp
from jax import lax
import jax.experimental.pallas as pl
import jax.experimental.pallas.tpu as pltpu

H, DH, SK, D, F = 32, 192, 32768, 640, 1536
W = min(4096, max(256, SK // 4))
BF = jnp.bfloat16
F32 = jnp.float32


def _ln(x32):
    m = jnp.mean(x32, axis=-1, keepdims=True)
    c = x32 - m
    v = jnp.mean(c * c, axis=-1, keepdims=True)
    mb = m.astype(BF).astype(F32)
    vb = v.astype(BF).astype(F32)
    num = (x32 - mb).astype(BF).astype(F32)
    den = (vb + 1e-5).astype(BF).astype(F32)
    den = jnp.sqrt(den).astype(BF).astype(F32)
    return (num / den).astype(BF)


def pieces(R, C, pr, pc, order="cr", r0=0):
    rs = [(r0 + r, min(pr, R - r)) for r in range(0, R, pr)]
    cs = [(c, min(pc, C - c)) for c in range(0, C, pc)]
    if order == "rc":
        return [(r, nr, c, nc) for (r, nr) in rs for (c, nc) in cs]
    return [(r, nr, c, nc) for (c, nc) in cs for (r, nr) in rs]


def merge(a, b):
    out, ia, ib = [], 0, 0
    while ia < len(a) or ib < len(b):
        if ib >= len(b) or (ia < len(a) and ia * len(b) <= ib * len(a)):
            out.append(a[ia]); ia += 1
        else:
            out.append(b[ib]); ib += 1
    return out


def split_even(lst, fracs):
    tot = sum(fracs)
    out, acc, prev = [], 0, 0
    for f in fracs:
        acc += f
        nxt = round(len(lst) * acc / tot)
        out.append(lst[prev:nxt]); prev = nxt
    return out


def make_kernel(R=3, kv_piece=(24, 512, "cr"), wq_piece=(8, 3072), wo_rows=24, w1_piece=(8, 1536), w2_rows=32,
                nq=4, n13=5, n2=4, plan=None, nosem=False, nocomp=False, pre="pair"):
    kvp = pieces(DH, W, *kv_piece)
    wqp = pieces(D, H * DH, *wq_piece, "rc")
    wop = pieces(H * DH, D, wo_rows, D, "rc")
    DC = D // n13
    FC = F // n2
    if plan is None:
        plan = {("c", H - 2): [0], ("c", H - 1): [1], ("ln", 0): [2], ("g", 0): [3], ("g", 1): [4], ("g", 2): [5, 6], ("g", 3): [7], ("g", 4): [8]}
    plan = dict(plan)
    assert sorted(sum(plan.values(), [])) == list(range(n13 + n2)), plan

    def dot(a, b_fn, shape, dims=(((1,), (0,)), ((), ())), tag="x"):
        if nocomp is True or (isinstance(nocomp, str) and tag in nocomp):
            return jnp.zeros(shape, F32)
        return lax.dot_general(a, b_fn(), dims, preferred_element_type=F32)

    def kernel(x_hbm, kt_hbm, vt_hbm, wq_hbm, wo_hbm, w1_hbm, w3_hbm, w2_hbm, o_ref,
               x_v, wq_v, q_v, kbuf, vbuf, wo_v, w1_v, w3_v, w2_v,
               sem_x, sem_wq, sem_k, sem_v, sem_wo, sem_w1, sem_w3, sem_w2):
        def cp2(src, dst, sem, p):
            r, nr, c, nc = p
            return pltpu.make_async_copy(src.at[pl.ds(r, nr), pl.ds(c, nc)], dst.at[pl.ds(r, nr), pl.ds(c, nc)], sem)
        def head_jobs(h, slot):
            ksrc = kt_hbm.at[h, :, pl.ds(SK - W, W)]
            vsrc = vt_hbm.at[h, :, pl.ds(SK - W, W)]
            jobs = []
            for p in kvp:
                jobs.append((ksrc, kbuf.at[slot], sem_k.at[slot], p, 0))
                jobs.append((vsrc, vbuf.at[slot], sem_v.at[slot], p, 1))
            return jobs
        def run_jobs(jobs):
            for (a, b, s_, p, pr) in jobs:
                cp2(a, b, s_, p).start(priority=pr)
        def wait_all(ref, sem):
            pltpu.make_async_copy(ref, ref, sem).wait()

        pltpu.make_async_copy(x_hbm, x_v, sem_x).start()
        if pre == "pair":
            run_jobs(merge([(wq_hbm, wq_v, sem_wq, p, 0) for p in wqp], [(wo_hbm, wo_v, sem_wo, p, 1) for p in wop]))
            prejobs = []
        else:
            hq, ho = len(wqp) // 2, len(wop) // 2
            run_jobs(merge([(wq_hbm, wq_v, sem_wq, p, 0) for p in wqp[:hq]], [(wq_hbm, wq_v, sem_wq, p, 1) for p in wqp[hq:]]))
            prejobs = merge([(wo_hbm, wo_v, sem_wo, p, 0) for p in wop[:ho]], [(wo_hbm, wo_v, sem_wo, p, 1) for p in wop[ho:]])
        alljobs = prejobs
        for h in range(R):
            alljobs = alljobs + head_jobs(h, h)
        n0 = 72 * 1024 * 48 // (kv_piece[0] * kv_piece[1] * 2 * 1024) * 1
        n0 = min(len(alljobs), max(64, n0 + 8))
        run_jobs(alljobs[:n0])
        wait_all(x_v, sem_x)
        x32 = x_v[...].astype(F32)
        lnx = _ln(x32)
        lnx8 = jnp.broadcast_to(lnx, (8, D))
        wait_all(wq_v, sem_wq)
        groups = split_even(alljobs[n0:], [1] * nq)
        QC = H // nq
        fences = [(wo_v, sem_wo), (kbuf.at[0], sem_k.at[0]), (vbuf.at[0], sem_v.at[0])]
        fenced = set()
        for c in range(nq):
            qc = dot(lnx8, lambda: wq_v[:, c * QC * DH:(c + 1) * QC * DH], (8, QC * DH), tag='q')
            for j in range(QC):
                q_v[c * QC + j] = qc[:, j * DH:(j + 1) * DH]
            run_jobs(groups[c])
            if c < len(fences) and c < nq - 1 and c >= 1:
                wait_all(*fences[c - 1]); fenced.add(c - 1)
        if 0 not in fenced:
            wait_all(wo_v, sem_wo)

        scale = jnp.float32(DH ** -0.5).astype(BF).astype(F32)

        def head_compute(h, slot, attn, skip=()):
            if 1 not in skip: wait_all(kbuf.at[slot], sem_k.at[slot])
            if 2 not in skip: wait_all(vbuf.at[slot], sem_v.at[slot])
            qh = q_v[h].astype(BF)
            s = dot(qh, lambda: kbuf[slot], (8, W), tag='k')
            s = s.astype(BF).astype(F32)
            s = (s * scale).astype(BF).astype(F32)
            m = jnp.max(s, axis=-1, keepdims=True)
            e = jnp.exp((s - m).astype(BF).astype(F32)).astype(BF).astype(F32)
            l = jnp.sum(e, axis=-1, keepdims=True).astype(BF).astype(F32)
            p = (e / l).astype(BF)
            o = dot(p, lambda: vbuf[slot], (8, DH), (((1,), (1,)), ((), ())), tag='v')
            row = h * DH if isinstance(h, int) else pl.multiple_of(h * DH, DH)
            return attn + dot(o.astype(BF), lambda: wo_v[pl.ds(row, DH), :], (8, D), tag='o')

        attn = head_compute(0, 0, jnp.zeros((8, D), F32), skip=fenced)
        run_jobs(head_jobs(R, 0))

        def head(h, attn):
            slot = h % R
            attn = head_compute(h, slot, attn)
            run_jobs(head_jobs(h + R, slot))
            return attn

        attn = lax.fori_loop(1, H - R, head, attn)
        wch = []
        for c in range(n13):
            pp = pieces(DC, F, *w1_piece, "rc", r0=c * DC)
            wch.append(merge([(w1_hbm, w1_v, sem_w1.at[c], p, 0) for p in pp],
                             [(w3_hbm, w3_v, sem_w3.at[c], p, 1) for p in pp]))
        for c in range(n2):
            pp = pieces(FC, D, w2_rows, D, "rc", r0=c * FC)
            wch.append([(w2_hbm, w2_v, sem_w2.at[c], p, i % 2) for i, p in enumerate(pp)])
        done = set()
        def slot_jobs(key):
            for ch in plan.get(key, []):
                run_jobs(wch[ch]); done.add(ch)
        for i in range(R):
            h = H - R + i
            attn = head_compute(h, h % R, attn)
            slot_jobs(("c", h))
        hres = (x32 + attn.astype(BF).astype(F32)).astype(BF).astype(F32)
        lnh = _ln(hres)
        slot_jobs(("ln", 0))
        gate = up = None
        for c in range(n13):
            assert c in done
            rows = pl.ds(c * DC, DC)
            wait_all(w1_v.at[rows], sem_w1.at[c])
            wait_all(w3_v.at[rows], sem_w3.at[c])
            lc = lnh[:, c * DC:(c + 1) * DC]
            g_ = dot(lc, lambda: w1_v[c * DC:(c + 1) * DC, :], (8, F), tag='g')
            u_ = dot(lc, lambda: w3_v[c * DC:(c + 1) * DC, :], (8, F), tag='g')
            gate = g_ if gate is None else gate + g_
            up = u_ if up is None else up + u_
            slot_jobs(("g", c))
        assert len(done) == n13 + n2
        gate = gate.astype(BF).astype(F32)
        up = up.astype(BF).astype(F32)
        sg = jax.nn.sigmoid(gate).astype(BF).astype(F32)
        hm = ((gate * sg).astype(BF).astype(F32) * up).astype(BF)
        out = None
        for c in range(n2):
            wait_all(w2_v.at[pl.ds(c * FC, FC)], sem_w2.at[c])
            o_ = dot(hm[:, c * FC:(c + 1) * FC], lambda: w2_v[c * FC:(c + 1) * FC, :], (8, D), tag='d')
            out = o_ if out is None else out + o_
        res = hres + out.astype(BF).astype(F32)
        o_ref[...] = res[0:1, :].astype(o_ref.dtype)

    @jax.jit
    def run(A_x, A_k_cache, A_v_cache, A_wq, A_wo, B_x, B_w1, B_w3, B_w2):
        x = A_x.reshape(1, D)
        kt = jnp.swapaxes(A_k_cache.reshape(H, SK, DH), 1, 2)
        vt = jnp.swapaxes(A_v_cache.reshape(H, SK, DH), 1, 2)
        out = pl.pallas_call(
            kernel,
            out_shape=jax.ShapeDtypeStruct((1, D), BF),
            in_specs=[pl.BlockSpec(memory_space=pl.ANY)] * 8,
            out_specs=pl.BlockSpec(memory_space=pltpu.VMEM),
            scratch_shapes=[
                pltpu.VMEM((1, D), BF),
                pltpu.VMEM((D, H * DH), BF),
                pltpu.VMEM((H, 8, DH), F32),
                pltpu.VMEM((R, DH, W), BF),
                pltpu.VMEM((R, DH, W), BF),
                pltpu.VMEM((H * DH, D), BF),
                pltpu.VMEM((D, F), BF),
                pltpu.VMEM((D, F), BF),
                pltpu.VMEM((F, D), BF),
                pltpu.SemaphoreType.DMA(()),
                pltpu.SemaphoreType.DMA(()),
                pltpu.SemaphoreType.DMA((R,)),
                pltpu.SemaphoreType.DMA((R,)),
                pltpu.SemaphoreType.DMA(()),
                pltpu.SemaphoreType.DMA((n13,)),
                pltpu.SemaphoreType.DMA((n13,)),
                pltpu.SemaphoreType.DMA((n2,)),
            ],
            compiler_params=pltpu.CompilerParams(vmem_limit_bytes=100 * 1024 * 1024,
                                                 disable_semaphore_checks=nosem, disable_bounds_checks=nosem),
        )(x, kt, vt, A_wq, A_wo, B_w1, B_w3, B_w2)
        return out.reshape(1, 1, D)
    return run


pallas_sequential_preLN__sliding_block_cached__glu_gated_swiglu__decode_kernel = make_kernel(
    plan={('c', 29): [0, 1], ('c', 30): [2], ('c', 31): [3], ('g', 0): [4], ('g', 1): [5, 6], ('g', 2): [7], ('g', 3): [8]})
```

```python
import jax
import jax.numpy as jnp
import numpy as np
from jax import lax
import jax.experimental.pallas as pl
import jax.experimental.pallas.tpu as pltpu

H, DH, SK, D, F = 32, 192, 32768, 640, 1536
W = min(4096, max(256, SK // 4))
BF = jnp.bfloat16
F32 = jnp.float32


def _bf16_round(v):
    u = int(np.float32(v).view(np.uint32))
    u = (u + 0x7FFF + ((u >> 16) & 1)) & 0xFFFF0000
    return float(np.uint32(u).view(np.float32))


SCALE = _bf16_round(DH ** -0.5)
EPS = _bf16_round(1e-5)


def _r(x):
    return x.astype(BF).astype(F32)


def _layernorm(x32):
    m = jnp.mean(x32, axis=-1, keepdims=True)
    c = x32 - m
    v = jnp.mean(c * c, axis=-1, keepdims=True)
    num = _r(x32 - _r(m))
    den = _r(jnp.sqrt(_r(_r(v) + EPS)))
    return (num / den).astype(BF)


def _pieces2(rows, cols, pr, pc, col_major, r0=0):
    rs = [(r0 + r, min(pr, rows - r)) for r in range(0, rows, pr)]
    cs = [(c, min(pc, cols - c)) for c in range(0, cols, pc)]
    if col_major:
        return [(r, nr, c, nc) for (c, nc) in cs for (r, nr) in rs]
    return [(r, nr, c, nc) for (r, nr) in rs for (c, nc) in cs]


def _pieces3(groups, rows, cols, g, pr, pc):
    return [(a, min(g, groups - a), r, pr, c, min(pc, cols - c))
            for r in range(0, rows, pr) for c in range(0, cols, pc) for a in range(0, groups, g)]


def _merge(a, b):
    out, ia, ib = [], 0, 0
    while ia < len(a) or ib < len(b):
        if ib >= len(b) or (ia < len(a) and ia * len(b) <= ib * len(a)):
            out.append(a[ia])
            ia += 1
        else:
            out.append(b[ib])
            ib += 1
    return out


def _split(lst, n):
    return [lst[i * len(lst) // n:(i + 1) * len(lst) // n] for i in range(n)]


def make_kernel(R=3, kv_piece=(40, 512), wq_piece=(3, 8, 512), wo_piece=(1, 16, 640), w13_piece=(8, 1536),
                w2_rows=16, nq=2, n0=400, w2ch=(512, 384, 384, 256),
                plan=(("c", 29, (0, 1)), ("c", 30, (2,)), ("c", 31, (3,)),
                      ("g", 0, (4,)), ("g", 1, (5, 6)), ("g", 2, (7,)), ("g", 3, (8,)))):
    GQ, GO = 5, 8
    RQ, RO = D // GQ, H * DH // GO
    HPG = H // GO
    N13 = GQ
    DC = D // N13
    N2 = len(w2ch)
    w2off = [sum(w2ch[:i]) for i in range(N2)]
    plan = {(k, i): ch for (k, i, ch) in plan}

    kvp = _pieces2(DH, W, *kv_piece, col_major=True)
    wqp = _pieces3(GQ, RQ, H * DH, *wq_piece)
    half = len(wqp) // 2
    wqp = _merge([(p, 0) for p in wqp[:half]], [(p, 1) for p in wqp[half:]])
    wop = [(p, (i // 2) % 2) for i, p in enumerate(_pieces3(GO, RO, D, *wo_piece))]

    def kernel(x_hbm, kt_hbm, vt_hbm, wq_hbm, wo_hbm, w1_hbm, w3_hbm, w2_hbm, o_hbm,
               x_v, wq_v, q_v, kbuf, vbuf, wo_v, w13_v, w2_v, o_v, sem_o):

        def body(sem_x, sem_f, sem_wq, sem_k, sem_v, sem_wo, sem_w13, sem_w2):
            def copy(src, dst, sem, p):
                if len(p) == 4:
                    idx = (pl.ds(p[0], p[1]), pl.ds(p[2], p[3]))
                else:
                    idx = (pl.ds(p[0], p[1]), pl.ds(p[2], p[3]), pl.ds(p[4], p[5]))
                return pltpu.make_async_copy(src.at[idx], dst.at[idx], sem)

            def issue(jobs):
                for (src, dst, sem, p, thread) in jobs:
                    copy(src, dst, sem, p).start(priority=thread)

            def wait_all(ref, sem):
                pltpu.make_async_copy(ref, ref, sem).wait()

            def head_jobs(h, slot):
                ksrc = kt_hbm.at[h, :, pl.ds(SK - W, W)]
                vsrc = vt_hbm.at[h, :, pl.ds(SK - W, W)]
                jobs = []
                for p in kvp:
                    jobs.append((ksrc, kbuf.at[slot], sem_k.at[slot], p, 0))
                    jobs.append((vsrc, vbuf.at[slot], sem_v.at[slot], p, 1))
                return jobs

            x_copy = pltpu.make_async_copy(x_hbm, x_v, sem_x)
            x_copy.start()
            issue([(wq_hbm, wq_v, sem_f if p[2] == 0 else sem_wq, p, t) for p, t in wqp])
            wait_all(wq_v.at[:, pl.ds(0, wq_piece[1])], sem_f)
            jobs = [(wo_hbm, wo_v, sem_wo, p, t) for p, t in wop]
            for h in range(R):
                jobs += head_jobs(h, h)
            issue(jobs[:n0])

            x_copy.wait()
            x32 = x_v[...].astype(F32)
            lnx = jnp.broadcast_to(_layernorm(x32), (8, D))
            wait_all(wq_v.at[:, pl.ds(wq_piece[1], RQ - wq_piece[1])], sem_wq)
            QC = H // nq
            for c, group in enumerate(_split(jobs[n0:], nq)):
                wq_c = wq_v[:, :, c * QC * DH:(c + 1) * QC * DH].reshape(D, QC * DH)
                qc = jnp.dot(lnx, wq_c, preferred_element_type=F32)
                for j in range(QC):
                    q_v[c * QC + j] = qc[:, j * DH:(j + 1) * DH]
                issue(group)
            wait_all(wo_v, sem_wo)

            def head_compute(h, slot, attn):
                wait_all(kbuf.at[slot], sem_k.at[slot])
                wait_all(vbuf.at[slot], sem_v.at[slot])
                qh = q_v[h].astype(BF)
                s = jnp.dot(qh, kbuf[slot], preferred_element_type=F32)
                s = _r(_r(s) * SCALE)
                m = jnp.max(s, axis=-1, keepdims=True)
                e = _r(jnp.exp(_r(s - m)))
                l = _r(jnp.sum(e, axis=-1, keepdims=True))
                p = (e / l).astype(BF)
                o = lax.dot_general(p, vbuf[slot], (((1,), (1,)), ((), ())),
                                    preferred_element_type=F32)
                row = (h % HPG) * DH
                if not isinstance(h, int):
                    row = pl.multiple_of(row, DH)
                return attn + jnp.dot(o.astype(BF), wo_v[h // HPG, pl.ds(row, DH), :],
                                      preferred_element_type=F32)

            attn = head_compute(0, 0, jnp.zeros((8, D), F32))
            issue(head_jobs(R, 0))

            def head(h, attn):
                slot = h % R
                attn = head_compute(h, slot, attn)
                issue(head_jobs(h + R, slot))
                return attn

            attn = lax.fori_loop(1, H - R, head, attn)

            wch = []
            for c in range(N13):
                pp = _pieces2(DC, F, *w13_piece, col_major=False, r0=c * DC)
                wch.append(_merge([(w1_hbm, w13_v.at[0], sem_w13.at[c], p, 0) for p in pp],
                                  [(w3_hbm, w13_v.at[1], sem_w13.at[c], p, 1) for p in pp]))
            for c in range(N2):
                pp = _pieces2(w2ch[c], D, w2_rows, D, col_major=False, r0=w2off[c])
                wch.append([(w2_hbm, w2_v, sem_w2.at[c], p, i % 2) for i, p in enumerate(pp)])

            def issue_w(kind, i):
                for ch in plan.get((kind, i), ()):
                    issue(wch[ch])

            for h in range(H - R, H):
                attn = head_compute(h, h % R, attn)
                issue_w("c", h)
            hres = _r(x32 + _r(attn))
            lnh = _layernorm(hres)
            gate = up = None
            for c in range(N13):
                wait_all(w13_v.at[:, pl.ds(c * DC, DC)], sem_w13.at[c])
                lc = lnh[:, c * DC:(c + 1) * DC]
                g_ = jnp.dot(lc, w13_v[0, c * DC:(c + 1) * DC, :], preferred_element_type=F32)
                u_ = jnp.dot(lc, w13_v[1, c * DC:(c + 1) * DC, :], preferred_element_type=F32)
                gate = g_ if gate is None else gate + g_
                up = u_ if up is None else up + u_
                issue_w("g", c)
            gate, up = _r(gate), _r(up)
            hm = (_r(gate * _r(jax.nn.sigmoid(gate))) * up).astype(BF)
            out = None
            for c in range(N2):
                r0, nr = w2off[c], w2ch[c]
                wait_all(w2_v.at[pl.ds(r0, nr)], sem_w2.at[c])
                o_ = jnp.dot(hm[:, r0:r0 + nr], w2_v[r0:r0 + nr, :], preferred_element_type=F32)
                out = o_ if out is None else out + o_
            res = hres + _r(out)
            o_v[...] = res[0:1, :].astype(o_v.dtype)
            pltpu.make_async_copy(o_v, o_hbm, sem_o).start()

        dma = pltpu.SemaphoreType.DMA
        pl.run_scoped(body, dma(()), dma(()), dma(()), dma((R,)), dma((R,)), dma(()), dma((N13,)), dma((N2,)))
        pltpu.make_async_copy(o_v, o_hbm, sem_o).wait()

    @jax.jit
    def run(A_x, A_k_cache, A_v_cache, A_wq, A_wo, B_x, B_w1, B_w3, B_w2):
        del B_x
        x = A_x.reshape(1, D)
        kt = jnp.swapaxes(A_k_cache.reshape(H, SK, DH), 1, 2)
        vt = jnp.swapaxes(A_v_cache.reshape(H, SK, DH), 1, 2)
        out = pl.pallas_call(
            kernel,
            out_shape=jax.ShapeDtypeStruct((1, D), A_x.dtype),
            in_specs=[pl.BlockSpec(memory_space=pl.ANY)] * 8,
            out_specs=pl.BlockSpec(memory_space=pl.ANY),
            scratch_shapes=[
                pltpu.VMEM((1, D), BF),
                pltpu.VMEM((GQ, RQ, H * DH), BF),
                pltpu.VMEM((H, 8, DH), F32),
                pltpu.VMEM((R, DH, W), BF),
                pltpu.VMEM((R, DH, W), BF),
                pltpu.VMEM((GO, RO, D), BF),
                pltpu.VMEM((2, D, F), BF),
                pltpu.VMEM((F, D), BF),
                pltpu.VMEM((1, D), BF),
                pltpu.SemaphoreType.DMA(()),
            ],
            compiler_params=pltpu.CompilerParams(vmem_limit_bytes=64 * 1024 * 1024),
        )(x, kt, vt, A_wq.reshape(GQ, RQ, H * DH), A_wo.reshape(GO, RO, D), B_w1, B_w3, B_w2)
        return out.reshape(1, 1, D)

    return run


pallas_sequential_preLN__sliding_block_cached__glu_gated_swiglu__decode_kernel = make_kernel()
```
